```python
import os as _os
_os.environ.setdefault("JAX_PLATFORMS", "cpu")
import jax
import jax.numpy as jnp

def _softmax(x, axis=-1):
    return jax.nn.softmax(x, axis=axis)
def _gelu(x):
    return jax.nn.gelu(x, approximate=True)
def _silu(x):
    return jax.nn.silu(x)
def _sigmoid(x):
    return jax.nn.sigmoid(x)
def _layernorm(x, axis=-1, eps=1e-5):
    m = jnp.mean(x, axis=axis, keepdims=True)
    v = jnp.var(x, axis=axis, keepdims=True)
    return (x - m) / jnp.sqrt(v + eps)
def _scatter_add(tgt, idx, src, axis=0):
    return tgt.at[idx].add(src)
def _segment_sum(src, seg, n):
    return jax.ops.segment_sum(src, seg, n)
class _Rng:
    def __init__(self, key):
        self._k = key
    def _next(self):
        self._k, sub = jax.random.split(self._k)
        return sub
    def normal(self, shape):
        return jax.random.normal(self._next(), shape, dtype=jnp.bfloat16)
    def randint(self, lo, hi, shape):
        return jax.random.randint(self._next(), shape, lo, hi, dtype=jnp.int32)
    def uniform(self, shape, lo=0.0, hi=1.0):
        return jax.random.uniform(self._next(), shape, jnp.bfloat16, lo, hi)
    def permutation(self, n):
        return jax.random.permutation(self._next(), n)


kernel_name = 'standalone__dense_activation_gelu__prompt'

def setup_inputs():
    _rng = _Rng(jax.random.key(int.from_bytes(__import__("os").urandom(4), "little")))
    _w = (lambda a: (lambda t: t.astype(jnp.bfloat16) if jnp.issubdtype(t.dtype, jnp.floating) else t)(jnp.asarray(a)))
    B, S, D, F = 1, 2048, 640, 1728
    return {
        "x": _w((lambda *s: _rng.normal(s) * 0.05)(B, S, D)),
        "w1": _w((lambda *s: _rng.normal(s) * 0.05)(D, F) * (D ** -0.5)),
        "b1": _w((lambda *s: _rng.normal(s) * 0.05)(F) * 0.01),
        "w2": _w((lambda *s: _rng.normal(s) * 0.05)(F, D) * (F ** -0.5)),
        "b2": _w((lambda *s: _rng.normal(s) * 0.05)(D) * 0.01),
    }

def reference(x, w1, b1, w2, b2):
    h = jnp.einsum("bsd,df->bsf", x, w1) + b1
    h = _gelu(h)
    return jnp.einsum("bsf,fd->bsd", h, w2) + b2
```

```python
import jax
import jax.numpy as jnp
from jax.experimental import pallas as pl
from jax.experimental.pallas import tpu as pltpu

_MXU = 128
_NT = (((1,), (1,)), ((), ()))


def _gelu_tanh(h):
    sqrt_2_over_pi = 0.7978845608028654
    inner = sqrt_2_over_pi * (h + 0.044715 * (h * h * h))
    return 0.5 * h * (1.0 + jnp.tanh(inner))


def _spans(sizes):
    out, start = [], 0
    for n in sizes:
        out.append((start, n))
        start += n
    return out


def _f_chunks(f):
    sizes, left = [], f
    for tiles in (1, 2, 4):
        n = tiles * _MXU
        if left <= n:
            break
        sizes.append(n)
        left -= n
    sizes.append(left)
    return sizes


def _row_tiles(m):
    big, last = 4 * _MXU, _MXU
    if m <= big + last:
        return [m]
    sizes, left = [], m - last
    while left > 0:
        n = min(big, left)
        sizes.append(n)
        left -= n
    sizes.append(last)
    return sizes


def _build_kernel(m, f, chunks, tiles, first_sub):
    n_ch, n_t = len(chunks), len(tiles)
    s_x, s_w1, s_w2 = 0, n_t, n_t + n_ch
    s_b1 = n_t + 2 * n_ch
    s_b2, s_out = s_b1 + 1, s_b1 + 2
    n_sem = s_out + n_t

    def kernel(x_hbm, w1t_hbm, b1_hbm, w2_hbm, b2_hbm, o_hbm,
               x_v, o_v, b1_v, b2_v, *rest):
        w1_v, w2_v, sem = rest[:n_ch], rest[n_ch:2 * n_ch], rest[2 * n_ch]

        def x_copy(t):
            a, n = tiles[t]
            return pltpu.make_async_copy(
                x_hbm.at[pl.ds(a, n), :], x_v.at[pl.ds(a, n), :], sem.at[s_x + t])

        def out_copy(t):
            a, n = tiles[t]
            return pltpu.make_async_copy(
                o_v.at[pl.ds(a, n), :], o_hbm.at[pl.ds(a, n), :], sem.at[s_out + t])

        def w1_copy(c):
            a, n = chunks[c]
            return pltpu.make_async_copy(
                w1t_hbm.at[pl.ds(a, n), :], w1_v[c], sem.at[s_w1 + c])

        def w2_copy(c):
            a, n = chunks[c]
            return pltpu.make_async_copy(
                w2_hbm.at[pl.ds(a, n), :], w2_v[c], sem.at[s_w2 + c])

        def b1_copy():
            return pltpu.make_async_copy(b1_hbm, b1_v, sem.at[s_b1])

        def b2_copy():
            return pltpu.make_async_copy(b2_hbm, b2_v, sem.at[s_b2])

        x_copy(0).start()
        w1_copy(0).start()
        b1_copy().start()
        w2_copy(0).start()
        for c in range(1, n_ch):
            w1_copy(c).start()
            w2_copy(c).start()
        b2_copy().start()
        for t in range(1, n_t):
            x_copy(t).start()

        def first_matmul(xs, w1t, swap_remainder):
            n = w1t.shape[0]
            n_main = (n // _MXU) * _MXU if swap_remainder else n
            parts = []
            if n_main:
                parts.append(jax.lax.dot_general(
                    xs, w1t[0:n_main], _NT, preferred_element_type=jnp.float32))
            if n_main < n:
                rem_t = jax.lax.dot_general(
                    w1t[n_main:n], xs, _NT, preferred_element_type=jnp.float32)
                parts.append(rem_t.T)
            return parts[0] if len(parts) == 1 else jnp.concatenate(parts, axis=1)

        def chunk_contribution(r0, rows, c, b1):
            a, n = chunks[c]
            h = first_matmul(x_v[r0:r0 + rows, :], w1_v[c][...], False)
            g = _gelu_tanh(h + b1[:, a:a + n]).astype(jnp.bfloat16)
            return jnp.dot(g, w2_v[c][...], preferred_element_type=jnp.float32)

        def full_tile(r0, rows, b1):
            w1t = jnp.concatenate([w1_v[c][...] for c in range(n_ch)], axis=0)
            w2 = jnp.concatenate([w2_v[c][...] for c in range(n_ch)], axis=0)
            h = first_matmul(x_v[r0:r0 + rows, :], w1t, True)
            g = _gelu_tanh(h + b1).astype(jnp.bfloat16)
            return jnp.dot(g, w2, preferred_element_type=jnp.float32)

        x_copy(0).wait()
        b1_copy().wait()
        b1 = b1_v[...].astype(jnp.float32)[None, :]

        a0, n0 = tiles[0]
        subs = [(r, min(first_sub, a0 + n0 - r)) for r in range(a0, a0 + n0, first_sub)]
        accs = [None] * len(subs)
        for c in range(n_ch):
            w1_copy(c).wait()
            w2_copy(c).wait()
            if c == n_ch - 1:
                b2_copy().wait()
            for j, (r0, rows) in enumerate(subs):
                p = chunk_contribution(r0, rows, c, b1)
                accs[j] = p if accs[j] is None else accs[j] + p
        b2 = b2_v[...].astype(jnp.float32)[None, :]
        for j, (r0, rows) in enumerate(subs):
            o_v[r0:r0 + rows, :] = (accs[j] + b2).astype(o_v.dtype)
        out_copy(0).start()

        for t in range(1, n_t):
            x_copy(t).wait()
        for t in range(1, n_t):
            a, n = tiles[t]
            o_v[a:a + n, :] = (full_tile(a, n, b1) + b2).astype(o_v.dtype)
            out_copy(t).start()

        for t in range(n_t):
            out_copy(t).wait()

    return kernel, n_sem


@jax.jit
def pallas_standalone__dense_activation_gelu__prompt_kernel(
    x: jax.Array,
    w1: jax.Array,
    b1: jax.Array,
    w2: jax.Array,
    b2: jax.Array,
):
    batch, seq, d = x.shape
    f = w1.shape[1]
    m = batch * seq
    dt = x.dtype

    chunks = _spans(_f_chunks(f))
    tiles = _spans(_row_tiles(m))
    kernel, n_sem = _build_kernel(m, f, chunks, tiles, first_sub=2 * _MXU)

    hbm = pl.BlockSpec(memory_space=pl.ANY)
    out = pl.pallas_call(
        kernel,
        in_specs=[hbm] * 5,
        out_specs=hbm,
        out_shape=jax.ShapeDtypeStruct((m, d), dt),
        scratch_shapes=(
            [pltpu.VMEM((m, d), dt),
             pltpu.VMEM((m, d), dt),
             pltpu.VMEM((f,), b1.dtype),
             pltpu.VMEM((d,), b2.dtype)]
            + [pltpu.VMEM((n, d), w1.dtype) for _, n in chunks]
            + [pltpu.VMEM((n, d), w2.dtype) for _, n in chunks]
            + [pltpu.SemaphoreType.DMA((n_sem,))]
        ),
        compiler_params=pltpu.CompilerParams(vmem_limit_bytes=100 * 1024 * 1024),
    )(x.reshape(m, d), w1.T, b1, w2, b2)
    return out.reshape(batch, seq, d)
```

```python
import jax
import jax.numpy as jnp
from jax.experimental import pallas as pl
from jax.experimental.pallas import tpu as pltpu

_MXU = 128
_NT = (((1,), (1,)), ((), ()))


def _gelu_tanh(h):
    sqrt_2_over_pi = 0.7978845608028654
    inner = sqrt_2_over_pi * (h + 0.044715 * (h * h * h))
    return 0.5 * h * (1.0 + jnp.tanh(inner))


def _spans(sizes):
    out, start = [], 0
    for n in sizes:
        out.append((start, n))
        start += n
    return out


def _f_chunks(f):
    sizes, left = [], f
    for tiles in (1, 2, 4):
        n = tiles * _MXU
        if left <= n:
            break
        sizes.append(n)
        left -= n
    sizes.append(left)
    return sizes


def _row_tiles(m):
    big, last = 4 * _MXU, _MXU
    if m <= big + last:
        return [m]
    sizes, left = [], m - last
    while left > 0:
        n = min(big, left)
        sizes.append(n)
        left -= n
    sizes.append(last)
    return sizes


def _build_kernel(chunks, tiles, first_sub):
    n_ch, n_t = len(chunks), len(tiles)
    s_x, s_w1, s_w2 = 0, n_t, n_t + n_ch
    s_b1 = n_t + 2 * n_ch
    s_b2, s_out = s_b1 + 1, s_b1 + 2
    n_sem = s_out + n_t

    def kernel(x_hbm, w1t_hbm, b1_hbm, w2_hbm, b2_hbm, o_hbm,
               x_v, o_v, b1_v, b2_v, *rest):
        w1_v, w2_v, sem = rest[:n_ch], rest[n_ch:2 * n_ch], rest[2 * n_ch]

        def x_copy(t):
            a, n = tiles[t]
            return pltpu.make_async_copy(
                x_hbm.at[pl.ds(a, n), :], x_v.at[pl.ds(a, n), :], sem.at[s_x + t])

        def out_copy(t):
            a, n = tiles[t]
            return pltpu.make_async_copy(
                o_v.at[pl.ds(a, n), :], o_hbm.at[pl.ds(a, n), :], sem.at[s_out + t])

        def w1_copy(c):
            a, n = chunks[c]
            return pltpu.make_async_copy(
                w1t_hbm.at[pl.ds(a, n), :], w1_v[c], sem.at[s_w1 + c])

        def w2_copy(c):
            a, n = chunks[c]
            return pltpu.make_async_copy(
                w2_hbm.at[pl.ds(a, n), :], w2_v[c], sem.at[s_w2 + c])

        def b1_copy():
            return pltpu.make_async_copy(b1_hbm, b1_v, sem.at[s_b1])

        def b2_copy():
            return pltpu.make_async_copy(b2_hbm, b2_v, sem.at[s_b2])

        x_copy(0).start()
        w1_copy(0).start()
        b1_copy().start()
        w2_copy(0).start()
        for c in range(1, n_ch):
            w1_copy(c).start()
            w2_copy(c).start()
        b2_copy().start()
        for t in range(1, n_t):
            x_copy(t).start()

        def first_matmul(xs, w1t):
            n = w1t.shape[0]
            n_main = (n // _MXU) * _MXU
            parts = []
            if n_main:
                parts.append(jax.lax.dot_general(
                    xs, w1t[0:n_main], _NT, preferred_element_type=jnp.float32))
            if n_main < n:
                rem_t = jax.lax.dot_general(
                    w1t[n_main:n], xs, _NT, preferred_element_type=jnp.float32)
                parts.append(rem_t.T)
            return parts[0] if len(parts) == 1 else jnp.concatenate(parts, axis=1)

        def chunk_contribution(r0, rows, c, b1):
            a, n = chunks[c]
            h = first_matmul(x_v[r0:r0 + rows, :], w1_v[c][...])
            g = _gelu_tanh(h + b1[:, a:a + n]).astype(jnp.bfloat16)
            return jnp.dot(g, w2_v[c][...], preferred_element_type=jnp.float32)

        def full_tile(r0, rows, b1):
            w1t = jnp.concatenate([w1_v[c][...] for c in range(n_ch)], axis=0)
            w2 = jnp.concatenate([w2_v[c][...] for c in range(n_ch)], axis=0)
            h = first_matmul(x_v[r0:r0 + rows, :], w1t)
            g = _gelu_tanh(h + b1).astype(jnp.bfloat16)
            return jnp.dot(g, w2, preferred_element_type=jnp.float32)

        x_copy(0).wait()
        b1_copy().wait()
        b1 = b1_v[...].astype(jnp.float32)[None, :]

        a0, n0 = tiles[0]
        subs = [(r, min(first_sub, a0 + n0 - r)) for r in range(a0, a0 + n0, first_sub)]
        accs = [None] * len(subs)
        for c in range(n_ch):
            w1_copy(c).wait()
            w2_copy(c).wait()
            if c == n_ch - 1:
                b2_copy().wait()
            for j, (r0, rows) in enumerate(subs):
                p = chunk_contribution(r0, rows, c, b1)
                accs[j] = p if accs[j] is None else accs[j] + p
        b2 = b2_v[...].astype(jnp.float32)[None, :]
        for j, (r0, rows) in enumerate(subs):
            o_v[r0:r0 + rows, :] = (accs[j] + b2).astype(o_v.dtype)
        out_copy(0).start()

        for t in range(1, n_t):
            x_copy(t).wait()
        for t in range(1, n_t):
            a, n = tiles[t]
            o_v[a:a + n, :] = (full_tile(a, n, b1) + b2).astype(o_v.dtype)
            out_copy(t).start()

        for t in range(n_t):
            out_copy(t).wait()

    return kernel, n_sem


@jax.jit
def pallas_standalone__dense_activation_gelu__prompt_kernel(
    x: jax.Array,
    w1: jax.Array,
    b1: jax.Array,
    w2: jax.Array,
    b2: jax.Array,
):
    batch, seq, d = x.shape
    f = w1.shape[1]
    m = batch * seq
    dt = x.dtype

    chunks = _spans(_f_chunks(f))
    tiles = _spans(_row_tiles(m))
    kernel, n_sem = _build_kernel(chunks, tiles, first_sub=2 * _MXU)

    hbm = pl.BlockSpec(memory_space=pl.ANY)
    out = pl.pallas_call(
        kernel,
        in_specs=[hbm] * 5,
        out_specs=hbm,
        out_shape=jax.ShapeDtypeStruct((m, d), dt),
        scratch_shapes=(
            [pltpu.VMEM((m, d), dt),
             pltpu.VMEM((m, d), dt),
             pltpu.VMEM((f,), b1.dtype),
             pltpu.VMEM((d,), b2.dtype)]
            + [pltpu.VMEM((n, d), w1.dtype) for _, n in chunks]
            + [pltpu.VMEM((n, d), w2.dtype) for _, n in chunks]
            + [pltpu.SemaphoreType.DMA((n_sem,))]
        ),
        compiler_params=pltpu.CompilerParams(vmem_limit_bytes=100 * 1024 * 1024),
    )(x.reshape(m, d), w1.T, b1, w2, b2)
    return out.reshape(batch, seq, d)
```
